```python
import os as _os
_os.environ.setdefault("JAX_PLATFORMS", "cpu")
import jax
import jax.numpy as jnp

def _softmax(x, axis=-1):
    return jax.nn.softmax(x, axis=axis)
def _gelu(x):
    return jax.nn.gelu(x, approximate=True)
def _silu(x):
    return jax.nn.silu(x)
def _sigmoid(x):
    return jax.nn.sigmoid(x)
def _layernorm(x, axis=-1, eps=1e-5):
    m = jnp.mean(x, axis=axis, keepdims=True)
    v = jnp.var(x, axis=axis, keepdims=True)
    return (x - m) / jnp.sqrt(v + eps)
def _scatter_add(tgt, idx, src, axis=0):
    return tgt.at[idx].add(src)
def _segment_sum(src, seg, n):
    return jax.ops.segment_sum(src, seg, n)
class _Rng:
    def __init__(self, key):
        self._k = key
    def _next(self):
        self._k, sub = jax.random.split(self._k)
        return sub
    def normal(self, shape):
        return jax.random.normal(self._next(), shape, dtype=jnp.bfloat16)
    def randint(self, lo, hi, shape):
        return jax.random.randint(self._next(), shape, lo, hi, dtype=jnp.int32)
    def uniform(self, shape, lo=0.0, hi=1.0):
        return jax.random.uniform(self._next(), shape, jnp.bfloat16, lo, hi)
    def permutation(self, n):
        return jax.random.permutation(self._next(), n)


kernel_name = 'sequential_preLN__softmax_full_mha__mixer_channel_mlp__prompt'

def setup_inputs():
    _rng = _Rng(jax.random.key(int.from_bytes(__import__("os").urandom(4), "little")))
    _w = (lambda a: (lambda t: t.astype(jnp.bfloat16) if jnp.issubdtype(t.dtype, jnp.floating) else t)(jnp.asarray(a)))
    def _A_setup():
        B, S, D = 1, 2048, 1024
        return {
            "x": _w((lambda *s: _rng.normal(s) * 0.05)(B, S, D)),
            "wqkv": _w((lambda *s: _rng.normal(s) * 0.05)(D, 3 * D)),
            "wo": _w((lambda *s: _rng.normal(s) * 0.05)(D, D)),
        }
    _A_in = _A_setup()

    def _B_setup():
        B, S, D, F = 1, 2048, 1024, 3584
        return {
            "x": _w((lambda *s: _rng.normal(s) * 0.05)(B, S, D)),
            "w1": _w((lambda *s: _rng.normal(s) * 0.8)(D, F) * (D ** -0.5)),
            "b1": _w((lambda *s: _rng.normal(s) * 0.8)(F)),
            "w2": _w((lambda *s: _rng.normal(s) * 0.8)(F, D) * (F ** -0.5)),
            "b2": _w((lambda *s: _rng.normal(s) * 0.05)(D)),
        }
    _B_in = _B_setup()

    return {
        "A_x": _A_in["x"],
        "A_wqkv": _A_in["wqkv"],
        "A_wo": _A_in["wo"],
        "B_x": _B_in["x"],
        "B_w1": _B_in["w1"],
        "B_b1": _B_in["b1"],
        "B_w2": _B_in["w2"],
        "B_b2": _B_in["b2"],
    }

def reference(A_x, A_wqkv, A_wo, B_x, B_w1, B_b1, B_w2, B_b2):
    def _A_ref(x, wqkv, wo):
        B, S, D = x.shape
        H = 32; Dh = D // H
        qkv = (lambda x, *d: x.transpose(*d))((x @ wqkv).reshape(B, S, 3, H, Dh), 2, 0, 3, 1, 4)
        q, k, v = qkv[0], qkv[1], qkv[2]
        scale = Dh ** -0.5
        scores = jnp.einsum("bhqd,bhkd->bhqk", q, k) * scale
        p = _softmax(scores, axis=-1)
        o = jnp.einsum("bhqk,bhkd->bhqd", p, v)
        return (lambda x, *d: x.transpose(*d))(o, 0, 2, 1, 3).reshape(B, S, D) @ wo

    def _B_ref(x, w1, b1, w2, b2):
        y = _layernorm(x, axis=-1)
        h = _gelu(jnp.einsum("bsd,df->bsf", y, w1) + b1)
        return jnp.einsum("bsf,fd->bsd", h, w2) + b2

    x = A_x
    h = x + _A_ref(_layernorm(x, axis=-1), A_wqkv, A_wo)
    h2 = h + _B_ref(_layernorm(h, axis=-1), B_w1, B_b1, B_w2, B_b2)
    return h2
```

```python
import math
import jax
import jax.numpy as jnp
from jax import lax
import jax.experimental.pallas as pl
import jax.experimental.pallas.tpu as pltpu

S = 2048
D = 1024
H = 32
DH = 32
F = 3584
EPS = 1e-5
NT = (((1,), (1,)), ((), ()))
QSCALE = (DH ** -0.5) * math.log2(math.e)

TX = 256
NX = S // TX
SUB = 128
WC = 512
NWC = 3 * D // WC
TB = 1024
TQ = 512
NSUB = S // TQ
TK = 128
NC = S // TK
TM3 = 128
N3 = S // TM3
TF = 896
A1_SLOT = 0
A2_SLOT = 1


def _ln(x):
    m = jnp.mean(x, axis=-1, keepdims=True)
    xc = x - m
    v = jnp.mean(xc * xc, axis=-1, keepdims=True)
    return xc * lax.rsqrt(v + EPS)


def _kernel(x_hbm, wqkv_hbm, wo_hbm, w1_hbm, b1_ref, w2_hbm, b2_ref, out_hbm,
            x_v, xn_v, xs_v, wqkv_v, wo_v, w1_v, w2_v, qkv_v, vt_v, ot_v, s_v, m_v,
            y_v, h_v, o_v, b1_v, b2_v, x_sems, w_sems, in_sems, out_sems):
    f32 = jnp.float32
    bf16 = jnp.bfloat16

    def x_copy(i):
        rows = pl.ds(pl.multiple_of(i * TX, TX), TX)
        return pltpu.make_async_copy(x_hbm.at[rows, :], x_v.at[rows, :], x_sems.at[i])

    def w_copy(j):
        cols = pl.ds(pl.multiple_of(j * WC, WC), WC)
        return pltpu.make_async_copy(wqkv_hbm.at[:, cols], wqkv_v.at[:, cols], w_sems.at[j])

    cp_wo = pltpu.make_async_copy(wo_hbm, wo_v, in_sems.at[0])
    cp_w1 = pltpu.make_async_copy(w1_hbm, w1_v, in_sems.at[1])
    cp_w2 = pltpu.make_async_copy(w2_hbm, w2_v, in_sems.at[2])

    x_copy(0).start()
    w_copy(0).start()

    for c in range(F // 128):
        b1_v[:, c * 128:(c + 1) * 128] = b1_ref[c:c + 1, :].astype(f32)
    for c in range(D // 128):
        b2_v[:, c * 128:(c + 1) * 128] = b2_ref[c:c + 1, :].astype(f32)

    def ln_rows(r0):
        rows = pl.ds(pl.multiple_of(r0, SUB), SUB)
        xn = _ln(x_v[rows, :].astype(f32)).astype(bf16)
        xn_v[rows, :] = xn
        return xn

    x_copy(0).wait()
    x_copy(1).start()
    xs_v[...] = ln_rows(0)
    w_copy(0).wait()

    def p1a(i, c):
        @pl.when(i + 1 < NX)
        def _():
            x_copy(i + 1).wait()
        @pl.when(i + 2 < NX)
        def _():
            x_copy(i + 2).start()
        @pl.when(i == NX - 3)
        def _():
            w_copy(1).start()
        xn = xs_v[...]
        for u in range(TX // SUB):
            r0 = i * TX + u * SUB
            rows = pl.ds(pl.multiple_of(r0, SUB), SUB)
            r = jnp.dot(xn, wqkv_v[:, 0:WC], preferred_element_type=f32)
            r = (r * QSCALE).astype(bf16)
            for g in range(WC // 128):
                qkv_v[g, rows, :] = r[:, g * 128:(g + 1) * 128]
            xn = ln_rows(jnp.minimum(r0 + SUB, S - SUB))
        xs_v[...] = xn
        return c
    lax.fori_loop(0, NX, p1a, 0)

    for j in range(2, NWC):
        w_copy(j).start()

    nb = S // TB
    def p1b(t, c):
        j = t // nb + 1
        i = t % nb
        @pl.when(i == 0)
        def _():
            w_copy(j).wait()
        @pl.when(t == 2)
        def _():
            cp_wo.start(); cp_w1.start(); cp_w2.start()
        scale = jnp.where(j < D // WC, QSCALE, 1.0).astype(f32)
        rows = pl.ds(pl.multiple_of(i * TB, TB), TB)
        cols = pl.ds(pl.multiple_of(j * WC, WC), WC)
        r = jnp.dot(xn_v[rows, :], wqkv_v[:, cols], preferred_element_type=f32)
        r = (r * scale).astype(bf16)
        for g in range(WC // 128):
            qkv_v[j * (WC // 128) + g, rows, :] = r[:, g * 128:(g + 1) * 128]
        return c
    lax.fori_loop(0, (NWC - 1) * nb, p1b, 0)

    lane = lax.broadcasted_iota(jnp.int32, (TQ, 128), 1) // DH

    def qmask(h, t):
        qg = qkv_v[h // 4, pl.ds(pl.multiple_of(t * TQ, TQ), TQ), :]
        return h // 4 + 8, jnp.where(lane == (h % 4), qg, jnp.zeros_like(qg))

    def att_sub(h, t, do_pv):
        if do_pv:
            hoff = pl.multiple_of(h * DH, DH)
            m = m_v[t]
        koff, qm = qmask(h + 1, t)
        mx = None; ls = []; ot = None
        for c in range(NC):
            rows = pl.ds(c * TK, TK)
            if do_pv:
                sc = s_v[t, rows, :]
                mm = m
                if c >= 2:
                    mm = m + jnp.minimum(ls[c - 2], 0.0)
                p = jnp.exp2(sc.reshape(TK // 8, 8, TQ) - mm[None])
                cl = jnp.sum(p, axis=0)
                ls.append(cl if c == 0 else ls[-1] + cl)
                o = jnp.dot(vt_v[pl.ds(hoff, DH), rows], p.reshape(TK, TQ).astype(bf16),
                            preferred_element_type=f32)
                ot = o if ot is None else ot + o
            st = lax.dot_general(qkv_v[koff, rows, :], qm, NT, preferred_element_type=f32)
            cm = jnp.max(st.reshape(TK // 8, 8, TQ), axis=0)
            mx = cm if mx is None else jnp.maximum(mx, cm)
            s_v[t, rows, :] = st
        m_v[t] = jnp.broadcast_to(jnp.max(mx, axis=0, keepdims=True), (8, TQ))
        if do_pv:
            ot_v[pl.ds(hoff, DH), pl.ds(pl.multiple_of(t * TQ, TQ), TQ)] = (
                ot / jnp.sum(ls[-1], axis=0, keepdims=True)).astype(bf16)

    def p2a(t, c):
        rows = pl.ds(pl.multiple_of(t * TQ, TQ), TQ)
        for g in range(8):
            vt_v[g * 128:(g + 1) * 128, rows] = qkv_v[16 + g, rows, :].T
        att_sub(-1, t, False)
        return c
    lax.fori_loop(0, NSUB, p2a, 0)
    def p2(h, c):
        for t in range(NSUB):
            att_sub(h, t, True)
        return c
    lax.fori_loop(0, H - 1, p2, 0)

    cp_wo.wait(); cp_w1.wait(); cp_w2.wait()

    def out_copy(i, slot):
        rows = pl.ds(pl.multiple_of(i * TM3, TM3), TM3)
        return pltpu.make_async_copy(o_v.at[slot], out_hbm.at[rows, :], out_sems.at[slot])

    def stage_a1(i):
        t = i // (TQ // TM3)
        lanes = pl.ds(pl.multiple_of((i % (TQ // TM3)) * TM3, TM3), TM3)
        m = m_v[t, :, lanes]
        p = jnp.exp2(s_v[t, :, lanes].reshape(S // 8, 8, TM3) - m[None])
        l = jnp.sum(jnp.sum(p, axis=0), axis=0, keepdims=True)
        ot = jnp.dot(vt_v[D - DH:D, :], p.reshape(S, TM3).astype(bf16), preferred_element_type=f32)
        return (ot / l).astype(bf16)

    def stage_a2(i, ot_last):
        rows = pl.ds(pl.multiple_of(i * TM3, TM3), TM3)
        ot_full = jnp.concatenate([ot_v[0:D - DH, rows], ot_last], axis=0)
        o = ot_full.T
        h = x_v[rows, :].astype(f32) + jnp.dot(o, wo_v[...], preferred_element_type=f32)
        y_v[...] = _ln(_ln(h)).astype(bf16)
        h_v[...] = h + b2_v[...]

    def stage_a(i):
        stage_a2(i, stage_a1(i))

    def p3(i, c):
        slot = i % 2
        @pl.when(i >= 2)
        def _():
            out_copy(i - 2, slot).wait()
        y = y_v[...]
        acc = h_v[...]
        nxt = jnp.minimum(i + 1, N3 - 1)
        for j in range(F // TF):
            cols = pl.ds(j * TF, TF)
            a = jnp.dot(y, w1_v[:, cols], preferred_element_type=f32)
            a = jax.nn.gelu(a + b1_v[:, cols], approximate=True).astype(bf16)
            acc = acc + jnp.dot(a, w2_v[cols, :], preferred_element_type=f32)
            if j == A1_SLOT:
                ot_last = stage_a1(nxt)
            if j == A2_SLOT:
                stage_a2(nxt, ot_last)
        o_v[slot] = acc.astype(bf16)
        out_copy(i, slot).start()
        return c
    stage_a(0)
    lax.fori_loop(0, N3, p3, 0)
    out_copy(N3 - 2, (N3 - 2) % 2).wait()
    out_copy(N3 - 1, (N3 - 1) % 2).wait()


@jax.jit
def pallas_sequential_preLN__softmax_full_mha__mixer_channel_mlp__prompt_kernel(
    A_x: jax.Array,
    A_wqkv: jax.Array,
    A_wo: jax.Array,
    B_x: jax.Array,
    B_w1: jax.Array,
    B_b1: jax.Array,
    B_w2: jax.Array,
    B_b2: jax.Array,
):
    x = A_x.reshape(S, D)
    bf = jnp.bfloat16
    any_spec = pl.BlockSpec(memory_space=pl.ANY)
    vmem_spec = pl.BlockSpec(memory_space=pltpu.VMEM)
    out = pl.pallas_call(
        _kernel,
        out_shape=jax.ShapeDtypeStruct((S, D), bf),
        in_specs=[any_spec, any_spec, any_spec, any_spec, vmem_spec, any_spec, vmem_spec],
        out_specs=any_spec,
        scratch_shapes=[
            pltpu.VMEM((S, D), bf),
            pltpu.VMEM((S, D), bf),
            pltpu.VMEM((SUB, D), bf),
            pltpu.VMEM((D, 3 * D), bf),
            pltpu.VMEM((D, D), bf),
            pltpu.VMEM((D, F), bf),
            pltpu.VMEM((F, D), bf),
            pltpu.VMEM((24, S, 128), bf),
            pltpu.VMEM((D, S), bf),
            pltpu.VMEM((D, S), bf),
            pltpu.VMEM((NSUB, S, TQ), jnp.float32),
            pltpu.VMEM((NSUB, 8, TQ), jnp.float32),
            pltpu.VMEM((TM3, D), bf),
            pltpu.VMEM((TM3, D), jnp.float32),
            pltpu.VMEM((2, TM3, D), bf),
            pltpu.VMEM((1, F), jnp.float32),
            pltpu.VMEM((1, D), jnp.float32),
            pltpu.SemaphoreType.DMA((NX,)),
            pltpu.SemaphoreType.DMA((NWC,)),
            pltpu.SemaphoreType.DMA((3,)),
            pltpu.SemaphoreType.DMA((2,)),
        ],
        compiler_params=pltpu.CompilerParams(vmem_limit_bytes=110 * 1024 * 1024, internal_scratch_in_bytes=65536),
    )(x, A_wqkv, A_wo, B_w1, B_b1.reshape(F // 128, 128), B_w2, B_b2.reshape(D // 128, 128))
    return out.reshape(1, S, D)
```

```python
import math
import jax
import jax.numpy as jnp
from jax import lax
import jax.experimental.pallas as pl
import jax.experimental.pallas.tpu as pltpu

S = 2048
D = 1024
H = 32
DH = 32
F = 3584
EPS = 1e-5
NT = (((1,), (1,)), ((), ()))
QSCALE = (DH ** -0.5) * math.log2(math.e)

TX = 256
NX = S // TX
SUB = 128
WC = 512
NWC = 3 * D // WC
TB = 1024
TQ = 512
NSUB = S // TQ
TK = 128
NC = S // TK
TM3 = 128
N3 = S // TM3
TF = 896
HB = 2
PSTEP = 1
A2_SLOT = 6


def _ln(x):
    m = jnp.mean(x, axis=-1, keepdims=True)
    xc = x - m
    v = jnp.mean(xc * xc, axis=-1, keepdims=True)
    return xc * lax.rsqrt(v + EPS)


def _kernel(x_hbm, wqkv_hbm, wo_hbm, w1_hbm, b1_ref, w2_hbm, b2_ref, out_hbm,
            x_v, xn_v, xs_v, wqkv_v, wo_v, w1_v, w2_v, qkv_v, vt_v, ot_v, otl_v, s_v, m_v,
            y_v, h_v, hp_v, o_v, b1_v, b2_v, b1r_v, b2r_v, x_sems, w_sems, in_sems, out_sems):
    f32 = jnp.float32
    bf16 = jnp.bfloat16

    def x_copy(r0, n, k):
        rows = pl.ds(r0, n)
        return pltpu.make_async_copy(x_hbm.at[rows, :], x_v.at[rows, :], x_sems.at[k])

    def x_mid(i):
        return x_copy(pl.multiple_of(SUB + i * TX, SUB), TX, i + 1)

    def w_copy(c0, n, k):
        cols = pl.ds(c0, n)
        return pltpu.make_async_copy(wqkv_hbm.at[:, cols], wqkv_v.at[:, cols], w_sems.at[k])

    def w_chunk(j):
        return w_copy(pl.multiple_of(j * WC, WC), WC, j)

    cp_wo = pltpu.make_async_copy(wo_hbm, wo_v, in_sems.at[0])
    cp_w1 = pltpu.make_async_copy(w1_hbm, w1_v, in_sems.at[1])
    cp_w2 = pltpu.make_async_copy(w2_hbm, w2_v, in_sems.at[2])
    cp_b1 = pltpu.make_async_copy(b1_ref, b1r_v, in_sems.at[3])
    cp_b2 = pltpu.make_async_copy(b2_ref, b2r_v, in_sems.at[4])
    HW = WC // 2
    cp_xa = x_copy(0, TX, 0)
    cp_xb = x_copy(TX, SUB, 1)
    cp_xz = x_copy(S - SUB, SUB, NX)
    cp_w0a = w_copy(0, HW, 0)
    cp_w0b = w_copy(HW, HW, NWC)

    cp_xa.start(); cp_w0a.start(); cp_w0b.start(); cp_xb.start()
    x_mid(1).start()

    def ln_rows(r0):
        rows = pl.ds(pl.multiple_of(r0, SUB), SUB)
        xn = _ln(x_v[rows, :].astype(f32)).astype(bf16)
        xn_v[rows, :] = xn
        return xn

    def q_store(rows, g0, r):
        r = (r * QSCALE).astype(bf16)
        for g in range(r.shape[1] // 128):
            qkv_v[g0 + g, rows, :] = r[:, g * 128:(g + 1) * 128]

    cp_xa.wait()
    ln_rows(0)
    ln_rows(SUB)
    cp_w0a.wait()
    q_store(pl.ds(0, TX), 0, jnp.dot(xn_v[0:TX, :], wqkv_v[:, 0:HW], preferred_element_type=f32))
    cp_w0b.wait()
    cp_xb.wait()
    for i in range(2, NX - 1):
        x_mid(i).start()
    cp_xz.start()
    q_store(pl.ds(0, TX), HW // 128, jnp.dot(xn_v[0:TX, :], wqkv_v[:, HW:WC], preferred_element_type=f32))
    xs_v[...] = ln_rows(TX)

    def p1a(i, c):
        @pl.when(i < NX - 1)
        def _():
            x_mid(i).wait()
        @pl.when(i == NX - 1)
        def _():
            cp_xz.wait()
        @pl.when(i == 3)
        def _():
            for j in range(1, NWC):
                w_chunk(j).start()
        xn = xs_v[...]
        for u in range(TX // SUB):
            r0 = i * TX + u * SUB
            rows = pl.ds(pl.multiple_of(r0, SUB), SUB)
            q_store(rows, 0, jnp.dot(xn, wqkv_v[:, 0:WC], preferred_element_type=f32))
            xn = ln_rows(jnp.minimum(r0 + SUB, S - SUB))
        xs_v[...] = xn
        return c
    lax.fori_loop(1, NX, p1a, 0)

    nb = S // TB
    def p1b(t, c):
        j = t // nb + 1
        i = t % nb
        @pl.when(i == 0)
        def _():
            w_chunk(j).wait()
        @pl.when(t == 1)
        def _():
            cp_b1.start(); cp_b2.start(); cp_wo.start(); cp_w1.start(); cp_w2.start()
        scale = jnp.where(j < D // WC, QSCALE, 1.0).astype(f32)
        rows = pl.ds(pl.multiple_of(i * TB, TB), TB)
        cols = pl.ds(pl.multiple_of(j * WC, WC), WC)
        r = jnp.dot(xn_v[rows, :], wqkv_v[:, cols], preferred_element_type=f32)
        r = (r * scale).astype(bf16)
        for g in range(WC // 128):
            qkv_v[j * (WC // 128) + g, rows, :] = r[:, g * 128:(g + 1) * 128]
        return c
    lax.fori_loop(0, (NWC - 1) * nb, p1b, 0)

    cp_b1.wait(); cp_b2.wait()
    lane = lax.broadcasted_iota(jnp.int32, (TQ, 128), 1) // DH

    def qmask(h, t):
        qg = qkv_v[h // 4, pl.ds(pl.multiple_of(t * TQ, TQ), TQ), :]
        return h // 4 + 8, jnp.where(lane == (h % 4), qg, jnp.zeros_like(qg))

    def att_sub(h, t, b, do_pv):
        if do_pv:
            hoff = pl.multiple_of(h * DH, DH)
            m = m_v[b]
        koff, qm = qmask(h + HB, t)
        mx = None; ls = []; ot = None
        for c in range(NC):
            rows = pl.ds(c * TK, TK)
            if do_pv:
                sc = s_v[b, rows, :]
                mm = m
                if c >= 2:
                    mm = m + jnp.minimum(ls[c - 2], 0.0)
                p = jnp.exp2(sc.reshape(TK // 8, 8, TQ) - mm[None])
                cl = jnp.sum(p, axis=0)
                ls.append(cl if c == 0 else ls[-1] + cl)
                o = jnp.dot(vt_v[pl.ds(hoff, DH), rows], p.reshape(TK, TQ).astype(bf16),
                            preferred_element_type=f32)
                ot = o if ot is None else ot + o
            st = lax.dot_general(qkv_v[koff, rows, :], qm, NT, preferred_element_type=f32)
            cm = jnp.max(st.reshape(TK // 8, 8, TQ), axis=0)
            mx = cm if mx is None else jnp.maximum(mx, cm)
            s_v[b, rows, :] = st
        m_v[b] = jnp.broadcast_to(jnp.max(mx, axis=0, keepdims=True), (8, TQ))
        if do_pv:
            ot_v[pl.ds(hoff, DH), pl.ds(pl.multiple_of(t * TQ, TQ), TQ)] = (
                ot / jnp.sum(ls[-1], axis=0, keepdims=True)).astype(bf16)

    def p2a(t, c):
        rows = pl.ds(pl.multiple_of(t * TQ, TQ), TQ)
        for g in range(8):
            vt_v[g * 128:(g + 1) * 128, rows] = qkv_v[16 + g, rows, :].T
        for cc in range(F // 128):
            b1_v[:, cc * 128:(cc + 1) * 128] = b1r_v[cc:cc + 1, :].astype(f32)
        for cc in range(D // 128):
            b2_v[:, cc * 128:(cc + 1) * 128] = b2r_v[cc:cc + 1, :].astype(f32)
        for j in range(HB):
            att_sub(j - HB, t, j * NSUB + t, False)
        return c
    lax.fori_loop(0, NSUB, p2a, 0)
    def p2(b, c):
        for j in range(HB):
            for t in range(NSUB):
                att_sub(b * HB + j, t, j * NSUB + t, True)
        return c
    lax.fori_loop(0, H // HB - 1, p2, 0)

    cp_wo.wait(); cp_w1.wait(); cp_w2.wait()

    KP = D - 128
    NPIECE = HB * NC // PSTEP
    RCH = TQ // 128
    NPC = NPIECE // RCH
    PN = D // NPC

    def p25(t, c_):
        o_cur = [None]
        def piece(k):
            r, n = k // NPC, k % NPC
            rows = pl.ds(pl.multiple_of(t * TQ + r * 128, 128), 128)
            if n == 0:
                o_cur[0] = ot_v[0:KP, rows].T
            cols = pl.ds(n * PN, PN)
            hp = jnp.dot(o_cur[0], wo_v[0:KP, cols], preferred_element_type=f32)
            hp_v[rows, cols] = hp + x_v[rows, cols].astype(f32)
        step = 0
        for j in range(HB):
            b = j * NSUB + t
            r0 = D - (HB - j) * DH
            m = m_v[b]
            ls = []; ot = None
            for c in range(NC):
                rows = pl.ds(c * TK, TK)
                sc = s_v[b, rows, :]
                mm = m
                if c >= 2:
                    mm = m + jnp.minimum(ls[c - 2], 0.0)
                p = jnp.exp2(sc.reshape(TK // 8, 8, TQ) - mm[None])
                cl = jnp.sum(p, axis=0)
                ls.append(cl if c == 0 else ls[-1] + cl)
                o = jnp.dot(vt_v[r0:r0 + DH, rows], p.reshape(TK, TQ).astype(bf16),
                            preferred_element_type=f32)
                ot = o if ot is None else ot + o
                if step % PSTEP == PSTEP - 1:
                    piece(step // PSTEP)
                step += 1
            otl_v[j * DH:(j + 1) * DH, pl.ds(pl.multiple_of(t * TQ, TQ), TQ)] = (
                ot / jnp.sum(ls[-1], axis=0, keepdims=True)).astype(bf16)
        return c_
    lax.fori_loop(0, NSUB, p25, 0)

    def out_copy(i, slot):
        rows = pl.ds(pl.multiple_of(i * TM3, TM3), TM3)
        return pltpu.make_async_copy(o_v.at[slot], out_hbm.at[rows, :], out_sems.at[slot])

    def stage_a(i):
        rows = pl.ds(pl.multiple_of(i * TM3, TM3), TM3)
        o = jnp.concatenate([ot_v[KP:D - HB * DH, rows], otl_v[:, rows]], axis=0).T
        h = hp_v[rows, :] + jnp.dot(o, wo_v[KP:D, :], preferred_element_type=f32)
        y_v[...] = _ln(_ln(h)).astype(bf16)
        h_v[...] = h + b2_v[...]

    def p3(i, c):
        slot = i % 2
        @pl.when(i >= 2)
        def _():
            out_copy(i - 2, slot).wait()
        y = y_v[...]
        acc = h_v[...]
        nxt = jnp.minimum(i + 1, N3 - 1)
        def hook(s):
            if s == A2_SLOT:
                stage_a(nxt)
        for j in range(F // TF):
            cols = pl.ds(j * TF, TF)
            a = jnp.dot(y, w1_v[:, cols], preferred_element_type=f32)
            a = jax.nn.gelu(a + b1_v[:, cols], approximate=True).astype(bf16)
            hook(2 * j)
            acc = acc + jnp.dot(a, w2_v[cols, :], preferred_element_type=f32)
            hook(2 * j + 1)
        o_v[slot] = acc.astype(bf16)
        out_copy(i, slot).start()
        return c
    stage_a(0)
    lax.fori_loop(0, N3, p3, 0)
    out_copy(N3 - 2, (N3 - 2) % 2).wait()
    out_copy(N3 - 1, (N3 - 1) % 2).wait()


@jax.jit
def pallas_sequential_preLN__softmax_full_mha__mixer_channel_mlp__prompt_kernel(
    A_x: jax.Array,
    A_wqkv: jax.Array,
    A_wo: jax.Array,
    B_x: jax.Array,
    B_w1: jax.Array,
    B_b1: jax.Array,
    B_w2: jax.Array,
    B_b2: jax.Array,
):
    x = A_x.reshape(S, D)
    bf = jnp.bfloat16
    any_spec = pl.BlockSpec(memory_space=pl.ANY)
    vmem_spec = pl.BlockSpec(memory_space=pltpu.VMEM)
    out = pl.pallas_call(
        _kernel,
        out_shape=jax.ShapeDtypeStruct((S, D), bf),
        in_specs=[any_spec] * 7,
        out_specs=any_spec,
        scratch_shapes=[
            pltpu.VMEM((S, D), bf),
            pltpu.VMEM((S, D), bf),
            pltpu.VMEM((SUB, D), bf),
            pltpu.VMEM((D, 3 * D), bf),
            pltpu.VMEM((D, D), bf),
            pltpu.VMEM((D, F), bf),
            pltpu.VMEM((F, D), bf),
            pltpu.VMEM((24, S, 128), bf),
            pltpu.VMEM((D, S), bf),
            pltpu.VMEM((D - HB * DH, S), bf),
            pltpu.VMEM((HB * DH, S), bf),
            pltpu.VMEM((HB * NSUB, S, TQ), jnp.float32),
            pltpu.VMEM((HB * NSUB, 8, TQ), jnp.float32),
            pltpu.VMEM((TM3, D), bf),
            pltpu.VMEM((TM3, D), jnp.float32),
            pltpu.VMEM((S, D), jnp.float32),
            pltpu.VMEM((2, TM3, D), bf),
            pltpu.VMEM((1, F), jnp.float32),
            pltpu.VMEM((1, D), jnp.float32),
            pltpu.VMEM((F // 128, 128), bf),
            pltpu.VMEM((D // 128, 128), bf),
            pltpu.SemaphoreType.DMA((NX + 1,)),
            pltpu.SemaphoreType.DMA((NWC + 1,)),
            pltpu.SemaphoreType.DMA((5,)),
            pltpu.SemaphoreType.DMA((2,)),
        ],
        compiler_params=pltpu.CompilerParams(vmem_limit_bytes=120 * 1024 * 1024, internal_scratch_in_bytes=65536),
    )(x, A_wqkv, A_wo, B_w1, B_b1.reshape(F // 128, 128), B_w2, B_b2.reshape(D // 128, 128))
    return out.reshape(1, S, D)
```

```python
import math
import jax
import jax.numpy as jnp
from jax import lax
import jax.experimental.pallas as pl
import jax.experimental.pallas.tpu as pltpu

S = 2048
D = 1024
H = 32
DH = 32
F = 3584
EPS = 1e-5
NT = (((1,), (1,)), ((), ()))
QSCALE = (DH ** -0.5) * math.log2(math.e)

TX = 256
NX = S // TX
SUB = 128
WC = 512
NWC = 3 * D // WC
TB = 1024
TQ = 512
NSUB = S // TQ
TK = 128
NC = S // TK
TM3 = 128
N3 = S // TM3
TF = 896
HB = 2
PSTEP = 1
A2_SLOT = 6
LAG = 2


def _ln(x):
    m = jnp.mean(x, axis=-1, keepdims=True)
    xc = x - m
    v = jnp.mean(xc * xc, axis=-1, keepdims=True)
    return xc * lax.rsqrt(v + EPS)


def _kernel(x_hbm, wqkv_hbm, wo_hbm, w1_hbm, b1_ref, w2_hbm, b2_ref, out_hbm,
            x_v, xn_v, xs_v, wqkv_v, wo_v, w1_v, w2_v, qkv_v, qt_v, qz_v, vt_v, ot_v, otl_v, s_v, m_v,
            y_v, h_v, hp_v, o_v, b1_v, b2_v, b1r_v, b2r_v, x_sems, w_sems, in_sems, out_sems):
    f32 = jnp.float32
    bf16 = jnp.bfloat16

    def x_copy(r0, n, k):
        rows = pl.ds(r0, n)
        return pltpu.make_async_copy(x_hbm.at[rows, :], x_v.at[rows, :], x_sems.at[k])

    def x_mid(i):
        return x_copy(pl.multiple_of(SUB + i * TX, SUB), TX, i + 1)

    def w_copy(c0, n, k):
        cols = pl.ds(c0, n)
        return pltpu.make_async_copy(wqkv_hbm.at[:, cols], wqkv_v.at[:, cols], w_sems.at[k])

    def w_chunk(j):
        return w_copy(pl.multiple_of(j * WC, WC), WC, j)

    cp_wo = pltpu.make_async_copy(wo_hbm, wo_v, in_sems.at[0])
    cp_w1 = pltpu.make_async_copy(w1_hbm, w1_v, in_sems.at[1])
    cp_w2 = pltpu.make_async_copy(w2_hbm, w2_v, in_sems.at[2])
    cp_b1 = pltpu.make_async_copy(b1_ref, b1r_v, in_sems.at[3])
    cp_b2 = pltpu.make_async_copy(b2_ref, b2r_v, in_sems.at[4])
    HW = WC // 2
    cp_xa = x_copy(0, TX, 0)
    cp_xb = x_copy(TX, SUB, 1)
    cp_xz = x_copy(S - SUB, SUB, NX)
    cp_w0a = w_copy(0, HW, 0)
    cp_w0b = w_copy(HW, HW, NWC)

    cp_xa.start(); cp_w0a.start(); cp_w0b.start(); cp_xb.start()
    x_mid(1).start()

    def ln_rows(r0):
        rows = pl.ds(pl.multiple_of(r0, SUB), SUB)
        xn = _ln(x_v[rows, :].astype(f32)).astype(bf16)
        xn_v[rows, :] = xn
        return xn

    def q_store(rows, g0, r):
        r = (r * QSCALE).astype(bf16)
        for g in range(r.shape[1] // 128):
            qkv_v[g0 + g, rows, :] = r[:, g * 128:(g + 1) * 128]

    cp_xa.wait()
    ln_rows(0)
    ln_rows(SUB)
    cp_w0a.wait()
    q_store(pl.ds(0, TX), 0, jnp.dot(xn_v[0:TX, :], wqkv_v[:, 0:HW], preferred_element_type=f32))
    cp_w0b.wait()
    cp_xb.wait()
    for i in range(2, NX - 1):
        x_mid(i).start()
    cp_xz.start()
    q_store(pl.ds(0, TX), HW // 128, jnp.dot(xn_v[0:TX, :], wqkv_v[:, HW:WC], preferred_element_type=f32))
    xs_v[...] = ln_rows(TX)

    def p1a(i, c):
        @pl.when(i < NX - 1)
        def _():
            x_mid(i).wait()
        @pl.when(i == NX - 1)
        def _():
            cp_xz.wait()
        @pl.when(i == 3)
        def _():
            for j in range(1, NWC):
                w_chunk(j).start()
        xn = xs_v[...]
        for u in range(TX // SUB):
            r0 = i * TX + u * SUB
            rows = pl.ds(pl.multiple_of(r0, SUB), SUB)
            q_store(rows, 0, jnp.dot(xn, wqkv_v[:, 0:WC], preferred_element_type=f32))
            xn = ln_rows(jnp.minimum(r0 + SUB, S - SUB))
        xs_v[...] = xn
        return c
    lax.fori_loop(1, NX, p1a, 0)

    nb = S // TB
    def p1b(t, c):
        j = t // nb + 1
        i = t % nb
        @pl.when(i == 0)
        def _():
            w_chunk(j).wait()
        @pl.when(t == 1)
        def _():
            cp_b1.start(); cp_b2.start(); cp_wo.start(); cp_w1.start(); cp_w2.start()
        scale = jnp.where(j < D // WC, QSCALE, 1.0).astype(f32)
        rows = pl.ds(pl.multiple_of(i * TB, TB), TB)
        cols = pl.ds(pl.multiple_of(j * WC, WC), WC)
        r = jnp.dot(xn_v[rows, :], wqkv_v[:, cols], preferred_element_type=f32)
        r = (r * scale).astype(bf16)
        for g in range(WC // 128):
            qkv_v[j * (WC // 128) + g, rows, :] = r[:, g * 128:(g + 1) * 128]
        return c
    lax.fori_loop(0, (NWC - 1) * nb, p1b, 0)

    cp_b1.wait(); cp_b2.wait()
    lane = lax.broadcasted_iota(jnp.int32, (TQ, 128), 1) // DH

    def qmask(h, t):
        qg = qkv_v[h // 4, pl.ds(pl.multiple_of(t * TQ, TQ), TQ), :]
        return h // 4 + 8, jnp.where(lane == (h % 4), qg, jnp.zeros_like(qg))

    ZP = 128 - DH

    def stage_q(h, t, b):
        cols = pl.ds(pl.multiple_of(t * TQ, TQ), TQ)
        qz_v[b, ZP:128, :] = qt_v[pl.ds(pl.multiple_of(h * DH, DH), DH), cols]

    def att_sub(h, t, b, do_pv):
        hn = h + HB
        if do_pv:
            hoff = pl.multiple_of(h * DH, DH)
            m = m_v[b]
            koff = hn // 4 + 8
            wstart = pl.multiple_of(ZP - DH * (hn % 4), DH)
        else:
            koff, qm = qmask(hn, t)
        mx = None; ls = []; ot = None
        for c in range(NC):
            rows = pl.ds(c * TK, TK)
            if do_pv:
                sc = s_v[b, rows, :]
                mm = m
                if c >= LAG:
                    mm = m + jnp.minimum(ls[c - LAG], 0.0)
                p = jnp.exp2(sc.reshape(TK // 8, 8, TQ) - mm[None])
                cl = jnp.sum(p, axis=0)
                ls.append(cl if c == 0 else ls[-1] + cl)
                o = jnp.dot(vt_v[pl.ds(hoff, DH), rows], p.reshape(TK, TQ).astype(bf16),
                            preferred_element_type=f32)
                ot = o if ot is None else o + ot
                st = jnp.dot(qkv_v[koff, rows, :], qz_v[b, pl.ds(wstart, 128), :],
                             preferred_element_type=f32)
            else:
                st = lax.dot_general(qkv_v[koff, rows, :], qm, NT, preferred_element_type=f32)
            cm = jnp.max(st.reshape(TK // 8, 8, TQ), axis=0)
            mx = cm if mx is None else jnp.maximum(mx, cm)
            s_v[b, rows, :] = st
        m_v[b] = jnp.broadcast_to(jnp.max(mx, axis=0, keepdims=True), (8, TQ))
        if do_pv:
            ot_v[pl.ds(hoff, DH), pl.ds(pl.multiple_of(t * TQ, TQ), TQ)] = (
                ot / jnp.sum(ls[-1], axis=0, keepdims=True)).astype(bf16)

    def p2a(t, c):
        rows = pl.ds(pl.multiple_of(t * TQ, TQ), TQ)
        for g in range(8):
            qt_v[g * 128:(g + 1) * 128, rows] = qkv_v[g, rows, :].T
        for g in range(8):
            vt_v[g * 128:(g + 1) * 128, rows] = qkv_v[16 + g, rows, :].T
        for cc in range(F // 128):
            b1_v[:, cc * 128:(cc + 1) * 128] = b1r_v[cc:cc + 1, :].astype(f32)
        for cc in range(D // 128):
            b2_v[:, cc * 128:(cc + 1) * 128] = b2r_v[cc:cc + 1, :].astype(f32)
        for j in range(HB):
            att_sub(j - HB, t, j * NSUB + t, False)
        for j in range(HB):
            b = j * NSUB + t
            qz_v[b, 0:ZP, :] = jnp.zeros((ZP, TQ), bf16)
            qz_v[b, 128:128 + ZP, :] = jnp.zeros((ZP, TQ), bf16)
            stage_q(HB + j, t, b)
        return c
    lax.fori_loop(0, NSUB, p2a, 0)
    def p2(b, c):
        for j in range(HB):
            for t in range(NSUB):
                att_sub(b * HB + j, t, j * NSUB + t, True)
        for j in range(HB):
            for t in range(NSUB):
                stage_q(jnp.minimum(b * HB + j + 2 * HB, H - 1), t, j * NSUB + t)
        return c
    lax.fori_loop(0, H // HB - 1, p2, 0)

    cp_wo.wait(); cp_w1.wait(); cp_w2.wait()

    KP = D - 128
    NPIECE = HB * NC // PSTEP
    RCH = TQ // 128
    NPC = NPIECE // RCH
    PN = D // NPC

    def p25(t, c_):
        o_cur = [None]
        def piece(k):
            r, n = k // NPC, k % NPC
            rows = pl.ds(pl.multiple_of(t * TQ + r * 128, 128), 128)
            if n == 0:
                o_cur[0] = ot_v[0:KP, rows].T
            cols = pl.ds(n * PN, PN)
            hp = jnp.dot(o_cur[0], wo_v[0:KP, cols], preferred_element_type=f32)
            hp_v[rows, cols] = hp + x_v[rows, cols].astype(f32)
        step = 0
        for j in range(HB):
            b = j * NSUB + t
            r0 = D - (HB - j) * DH
            m = m_v[b]
            ls = []; ot = None
            for c in range(NC):
                rows = pl.ds(c * TK, TK)
                sc = s_v[b, rows, :]
                mm = m
                if c >= 2:
                    mm = m + jnp.minimum(ls[c - 2], 0.0)
                p = jnp.exp2(sc.reshape(TK // 8, 8, TQ) - mm[None])
                cl = jnp.sum(p, axis=0)
                ls.append(cl if c == 0 else ls[-1] + cl)
                o = jnp.dot(vt_v[r0:r0 + DH, rows], p.reshape(TK, TQ).astype(bf16),
                            preferred_element_type=f32)
                ot = o if ot is None else o + ot
                if step % PSTEP == PSTEP - 1:
                    piece(step // PSTEP)
                step += 1
            otl_v[j * DH:(j + 1) * DH, pl.ds(pl.multiple_of(t * TQ, TQ), TQ)] = (
                ot / jnp.sum(ls[-1], axis=0, keepdims=True)).astype(bf16)
        return c_
    lax.fori_loop(0, NSUB, p25, 0)

    def out_copy(i, slot):
        rows = pl.ds(pl.multiple_of(i * TM3, TM3), TM3)
        return pltpu.make_async_copy(o_v.at[slot], out_hbm.at[rows, :], out_sems.at[slot])

    def stage_a(i):
        rows = pl.ds(pl.multiple_of(i * TM3, TM3), TM3)
        o = jnp.concatenate([ot_v[KP:D - HB * DH, rows], otl_v[:, rows]], axis=0).T
        h = hp_v[rows, :] + jnp.dot(o, wo_v[KP:D, :], preferred_element_type=f32)
        y_v[...] = _ln(_ln(h)).astype(bf16)
        h_v[...] = h + b2_v[...]

    def p3(i, c):
        slot = i % 2
        @pl.when(i >= 2)
        def _():
            out_copy(i - 2, slot).wait()
        y = y_v[...]
        acc = h_v[...]
        nxt = jnp.minimum(i + 1, N3 - 1)
        def hook(s):
            if s == A2_SLOT:
                stage_a(nxt)
        for j in range(F // TF):
            cols = pl.ds(j * TF, TF)
            a = jnp.dot(y, w1_v[:, cols], preferred_element_type=f32)
            a = jax.nn.gelu(a + b1_v[:, cols], approximate=True).astype(bf16)
            hook(2 * j)
            acc = acc + jnp.dot(a, w2_v[cols, :], preferred_element_type=f32)
            hook(2 * j + 1)
        o_v[slot] = acc.astype(bf16)
        out_copy(i, slot).start()
        return c
    stage_a(0)
    lax.fori_loop(0, N3, p3, 0)
    out_copy(N3 - 2, (N3 - 2) % 2).wait()
    out_copy(N3 - 1, (N3 - 1) % 2).wait()


@jax.jit
def pallas_sequential_preLN__softmax_full_mha__mixer_channel_mlp__prompt_kernel(
    A_x: jax.Array,
    A_wqkv: jax.Array,
    A_wo: jax.Array,
    B_x: jax.Array,
    B_w1: jax.Array,
    B_b1: jax.Array,
    B_w2: jax.Array,
    B_b2: jax.Array,
):
    x = A_x.reshape(S, D)
    bf = jnp.bfloat16
    any_spec = pl.BlockSpec(memory_space=pl.ANY)
    vmem_spec = pl.BlockSpec(memory_space=pltpu.VMEM)
    out = pl.pallas_call(
        _kernel,
        out_shape=jax.ShapeDtypeStruct((S, D), bf),
        in_specs=[any_spec] * 7,
        out_specs=any_spec,
        scratch_shapes=[
            pltpu.VMEM((S, D), bf),
            pltpu.VMEM((S, D), bf),
            pltpu.VMEM((SUB, D), bf),
            pltpu.VMEM((D, 3 * D), bf),
            pltpu.VMEM((D, D), bf),
            pltpu.VMEM((D, F), bf),
            pltpu.VMEM((F, D), bf),
            pltpu.VMEM((24, S, 128), bf),
            pltpu.VMEM((D, S), bf),
            pltpu.VMEM((HB * NSUB, 128 + 128 - DH, TQ), bf),
            pltpu.VMEM((D, S), bf),
            pltpu.VMEM((D - HB * DH, S), bf),
            pltpu.VMEM((HB * DH, S), bf),
            pltpu.VMEM((HB * NSUB, S, TQ), jnp.float32),
            pltpu.VMEM((HB * NSUB, 8, TQ), jnp.float32),
            pltpu.VMEM((TM3, D), bf),
            pltpu.VMEM((TM3, D), jnp.float32),
            pltpu.VMEM((S, D), jnp.float32),
            pltpu.VMEM((2, TM3, D), bf),
            pltpu.VMEM((1, F), jnp.float32),
            pltpu.VMEM((1, D), jnp.float32),
            pltpu.VMEM((F // 128, 128), bf),
            pltpu.VMEM((D // 128, 128), bf),
            pltpu.SemaphoreType.DMA((NX + 1,)),
            pltpu.SemaphoreType.DMA((NWC + 1,)),
            pltpu.SemaphoreType.DMA((5,)),
            pltpu.SemaphoreType.DMA((2,)),
        ],
        compiler_params=pltpu.CompilerParams(vmem_limit_bytes=120 * 1024 * 1024, internal_scratch_in_bytes=65536),
    )(x, A_wqkv, A_wo, B_w1, B_b1.reshape(F // 128, 128), B_w2, B_b2.reshape(D // 128, 128))
    return out.reshape(1, S, D)
```

```python
import math

import jax
import jax.numpy as jnp
from jax import lax
import jax.experimental.pallas as pl
import jax.experimental.pallas.tpu as pltpu

S = 2048
D = 1024
H = 32
DH = 32
F = 3584
EPS = 1e-5
NT = (((1,), (1,)), ((), ()))
QSCALE = (DH ** -0.5) * math.log2(math.e)

TX = 256
NX = S // TX
SUB = 128
WC = 512
NWC = 3 * D // WC
TB = 1024
TQ = 512
NSUB = S // TQ
TK = 128
NC = S // TK
HB = 2
LAG = 2
ZP = 128 - DH
KP = D - 128
TM3 = 128
N3 = S // TM3
TF = 896
A2_SLOT = 6


def _ln(x):
    m = jnp.mean(x, axis=-1, keepdims=True)
    xc = x - m
    v = jnp.mean(xc * xc, axis=-1, keepdims=True)
    return xc * lax.rsqrt(v + EPS)


def _kernel(x_hbm, wqkv_hbm, wo_hbm, w1_hbm, b1_hbm, w2_hbm, b2_hbm, out_hbm,
            x_v, xn_v, xs_v, wqkv_v, wo_v, w1_v, w2_v, qkv_v, qt_v, qz_v, vt_v,
            ot_v, otl_v, og_v, s_v, m_v, y_v, h_v, hp_v, o_v, b1_v, b2_v,
            b1r_v, b2r_v, x_sems, w_sems, in_sems, out_sems):
    f32 = jnp.float32
    bf16 = jnp.bfloat16

    def x_copy(r0, n, k):
        rows = pl.ds(r0, n)
        return pltpu.make_async_copy(x_hbm.at[rows, :], x_v.at[rows, :], x_sems.at[k])

    def x_mid(i):
        return x_copy(pl.multiple_of(SUB + i * TX, SUB), TX, i + 1)

    def w_copy(c0, n, k):
        cols = pl.ds(c0, n)
        return pltpu.make_async_copy(wqkv_hbm.at[:, cols], wqkv_v.at[:, cols], w_sems.at[k])

    def w_chunk(j):
        return w_copy(pl.multiple_of(j * WC, WC), WC, j)

    cp_wo = pltpu.make_async_copy(wo_hbm, wo_v, in_sems.at[0])
    cp_w1 = pltpu.make_async_copy(w1_hbm, w1_v, in_sems.at[1])
    cp_w2 = pltpu.make_async_copy(w2_hbm, w2_v, in_sems.at[2])
    cp_b1 = pltpu.make_async_copy(b1_hbm, b1r_v, in_sems.at[3])
    cp_b2 = pltpu.make_async_copy(b2_hbm, b2r_v, in_sems.at[4])
    HW = WC // 2
    cp_xa = x_copy(0, TX, 0)
    cp_xb = x_copy(TX, SUB, 1)
    cp_xz = x_copy(S - SUB, SUB, NX)
    cp_w0a = w_copy(0, HW, 0)
    cp_w0b = w_copy(HW, HW, NWC)

    cp_xa.start(); cp_w0a.start(); cp_w0b.start(); cp_xb.start()
    x_mid(1).start()

    for b in range(HB * NSUB):
        qz_v[b, 0:ZP, :] = jnp.zeros((ZP, TQ), bf16)
        qz_v[b, 128:128 + ZP, :] = jnp.zeros((ZP, TQ), bf16)

    def ln_rows(r0):
        rows = pl.ds(pl.multiple_of(r0, SUB), SUB)
        xn = _ln(x_v[rows, :].astype(f32)).astype(bf16)
        xn_v[rows, :] = xn
        return xn

    def q_store(rows, g0, r):
        r = (r * QSCALE).astype(bf16)
        for g in range(r.shape[1] // 128):
            qkv_v[g0 + g, rows, :] = r[:, g * 128:(g + 1) * 128]

    cp_xa.wait()
    ln_rows(0)
    ln_rows(SUB)
    cp_w0a.wait()
    q_store(pl.ds(0, TX), 0,
            jnp.dot(xn_v[0:TX, :], wqkv_v[:, 0:HW], preferred_element_type=f32))
    cp_w0b.wait()
    cp_xb.wait()
    for i in range(2, NX - 1):
        x_mid(i).start()
    cp_xz.start()
    q_store(pl.ds(0, TX), HW // 128,
            jnp.dot(xn_v[0:TX, :], wqkv_v[:, HW:WC], preferred_element_type=f32))
    xs_v[...] = ln_rows(TX)

    def p1a(i, c):
        @pl.when(i < NX - 1)
        def _():
            x_mid(i).wait()

        @pl.when(i == NX - 1)
        def _():
            cp_xz.wait()

        @pl.when(i == 3)
        def _():
            for j in range(1, NWC):
                w_chunk(j).start()

        xn = xs_v[...]
        for u in range(TX // SUB):
            r0 = i * TX + u * SUB
            rows = pl.ds(pl.multiple_of(r0, SUB), SUB)
            q_store(rows, 0, jnp.dot(xn, wqkv_v[:, 0:WC], preferred_element_type=f32))
            xn = ln_rows(jnp.minimum(r0 + SUB, S - SUB))
        xs_v[...] = xn
        return c
    lax.fori_loop(1, NX, p1a, 0)

    nb = S // TB

    def p1b(t, c):
        j = t // nb + 1
        i = t % nb

        @pl.when(i == 0)
        def _():
            w_chunk(j).wait()

        @pl.when(t == 1)
        def _():
            cp_b1.start(); cp_b2.start(); cp_wo.start(); cp_w1.start(); cp_w2.start()

        scale = jnp.where(j < D // WC, QSCALE, 1.0).astype(f32)
        rows = pl.ds(pl.multiple_of(i * TB, TB), TB)
        cols = pl.ds(pl.multiple_of(j * WC, WC), WC)
        r = jnp.dot(xn_v[rows, :], wqkv_v[:, cols], preferred_element_type=f32)
        r = (r * scale).astype(bf16)
        for g in range(WC // 128):
            qkv_v[j * (WC // 128) + g, rows, :] = r[:, g * 128:(g + 1) * 128]
        return c
    lax.fori_loop(0, (NWC - 1) * nb, p1b, 0)

    cp_b1.wait(); cp_b2.wait()
    lane = lax.broadcasted_iota(jnp.int32, (TQ, 128), 1) // DH

    def stage_q(h, t, b):
        cols = pl.ds(pl.multiple_of(t * TQ, TQ), TQ)
        qz_v[b, ZP:128, :] = qt_v[pl.ds(pl.multiple_of(h * DH, DH), DH), cols]

    def softmax_pv_chunk(b, c, m, ls, ot, vrows):
        rows = pl.ds(c * TK, TK)
        sc = s_v[b, rows, :]

        def finish():
            mm = m
            if c >= LAG:
                mm = m + jnp.minimum(ls[c - LAG], 0.0)
            p = jnp.exp2(sc.reshape(TK // 8, 8, TQ) - mm[None])
            cl = jnp.sum(p, axis=0)
            ls.append(cl if c == 0 else ls[-1] + cl)
            o = jnp.dot(vt_v[vrows, rows], p.reshape(TK, TQ).astype(bf16),
                        preferred_element_type=f32)
            return o if ot is None else o + ot
        return finish

    def att_sub(h, t, b, do_pv, first=False):
        hn = h + HB
        koff = hn // 4 + 8
        if do_pv:
            hoff = pl.multiple_of(h * DH, DH)
            m = m_v[b]
            wstart = pl.multiple_of(ZP - DH * (hn % 4), DH)
        else:
            qg = qkv_v[hn // 4, pl.ds(pl.multiple_of(t * TQ, TQ), TQ), :]
            qm = jnp.where(lane == (hn % 4), qg, jnp.zeros_like(qg))
        mx = None
        ls = []
        ot = None
        for c in range(NC):
            rows = pl.ds(c * TK, TK)
            if do_pv:
                finish = softmax_pv_chunk(b, c, m, ls, ot, pl.ds(hoff, DH))
                qk_first = first and c == 0
                if qk_first:
                    st = jnp.dot(qkv_v[koff, rows, :], qz_v[b, pl.ds(wstart, 128), :],
                                 preferred_element_type=f32)
                ot = finish()
                if not qk_first:
                    st = jnp.dot(qkv_v[koff, rows, :], qz_v[b, pl.ds(wstart, 128), :],
                                 preferred_element_type=f32)
            else:
                st = lax.dot_general(qkv_v[koff, rows, :], qm, NT,
                                     preferred_element_type=f32)
            cm = jnp.max(st.reshape(TK // 8, 8, TQ), axis=0)
            mx = cm if mx is None else jnp.maximum(mx, cm)
            s_v[b, rows, :] = st
        m_v[b] = jnp.broadcast_to(jnp.max(mx, axis=0, keepdims=True), (8, TQ))
        if do_pv:
            ot_v[pl.ds(hoff, DH), pl.ds(pl.multiple_of(t * TQ, TQ), TQ)] = (
                ot / jnp.sum(ls[-1], axis=0, keepdims=True)).astype(bf16)

    def p2a(t, c):
        rows = pl.ds(pl.multiple_of(t * TQ, TQ), TQ)
        for g in range(8):
            qt_v[g * 128:(g + 1) * 128, rows] = qkv_v[g, rows, :].T
        for g in range(8):
            vt_v[g * 128:(g + 1) * 128, rows] = qkv_v[16 + g, rows, :].T
        for cc in range(F // 128):
            b1_v[:, cc * 128:(cc + 1) * 128] = b1r_v[cc:cc + 1, :].astype(f32)
        for cc in range(D // 128):
            b2_v[:, cc * 128:(cc + 1) * 128] = b2r_v[cc:cc + 1, :].astype(f32)
        for j in range(HB):
            att_sub(j - HB, t, j * NSUB + t, False)
        for j in range(HB):
            stage_q(HB + j, t, j * NSUB + t)
        return c
    lax.fori_loop(0, NSUB, p2a, 0)

    def p2(b, c):
        for j in range(HB):
            for t in range(NSUB):
                att_sub(b * HB + j, t, j * NSUB + t, True, first=(j == 0 and t == 0))
        for j in range(HB):
            for t in range(NSUB):
                stage_q(jnp.minimum(b * HB + j + 2 * HB, H - 1), t, j * NSUB + t)
        return c
    lax.fori_loop(0, H // HB - 1, p2, 0)

    cp_wo.wait(); cp_w1.wait(); cp_w2.wait()

    NPC = HB * NC // (TQ // 128)
    PN = D // NPC

    def pre_t(t):
        cols = pl.ds(pl.multiple_of(t * TQ, TQ), TQ)
        og_v[cols, :] = ot_v[0:KP, cols].T

    def p25(t, c_):
        o_cur = [None]

        def piece(k):
            r, n = k // NPC, k % NPC
            rows = pl.ds(pl.multiple_of(t * TQ + r * 128, 128), 128)
            if n == 0:
                o_cur[0] = og_v[rows, :]
            cols = pl.ds(n * PN, PN)
            hp = jnp.dot(o_cur[0], wo_v[0:KP, cols], preferred_element_type=f32)
            hp_v[rows, cols] = hp + x_v[rows, cols].astype(f32)

        for j in range(HB):
            b = j * NSUB + t
            r0 = D - (HB - j) * DH
            m = m_v[b]
            ls = []
            ot = None
            for c in range(NC):
                ot = softmax_pv_chunk(b, c, m, ls, ot, pl.ds(r0, DH))()
                piece(j * NC + c)
            otl_v[j * DH:(j + 1) * DH, pl.ds(pl.multiple_of(t * TQ, TQ), TQ)] = (
                ot / jnp.sum(ls[-1], axis=0, keepdims=True)).astype(bf16)
        pre_t(jnp.minimum(t + 1, NSUB - 1))
        return c_
    pre_t(0)
    lax.fori_loop(0, NSUB, p25, 0)

    def out_copy(i, slot):
        rows = pl.ds(pl.multiple_of(i * TM3, TM3), TM3)
        return pltpu.make_async_copy(o_v.at[slot], out_hbm.at[rows, :], out_sems.at[slot])

    def stage_a(i):
        rows = pl.ds(pl.multiple_of(i * TM3, TM3), TM3)
        o = jnp.concatenate([ot_v[KP:D - HB * DH, rows], otl_v[:, rows]], axis=0).T
        h = hp_v[rows, :] + jnp.dot(o, wo_v[KP:D, :], preferred_element_type=f32)
        y_v[...] = _ln(_ln(h)).astype(bf16)
        h_v[...] = h + b2_v[...]

    def p3(i, c):
        slot = i % 2

        @pl.when(i >= 2)
        def _():
            out_copy(i - 2, slot).wait()

        y = y_v[...]
        acc = h_v[...]
        nxt = jnp.minimum(i + 1, N3 - 1)
        for j in range(F // TF):
            cols = pl.ds(j * TF, TF)
            a = jnp.dot(y, w1_v[:, cols], preferred_element_type=f32)
            a = jax.nn.gelu(a + b1_v[:, cols], approximate=True).astype(bf16)
            if 2 * j == A2_SLOT:
                stage_a(nxt)
            acc = acc + jnp.dot(a, w2_v[cols, :], preferred_element_type=f32)
            if 2 * j + 1 == A2_SLOT:
                stage_a(nxt)
        o_v[slot] = acc.astype(bf16)
        out_copy(i, slot).start()
        return c
    stage_a(0)
    lax.fori_loop(0, N3, p3, 0)
    out_copy(N3 - 2, (N3 - 2) % 2).wait()
    out_copy(N3 - 1, (N3 - 1) % 2).wait()


@jax.jit
def pallas_sequential_preLN__softmax_full_mha__mixer_channel_mlp__prompt_kernel(
    A_x: jax.Array,
    A_wqkv: jax.Array,
    A_wo: jax.Array,
    B_x: jax.Array,
    B_w1: jax.Array,
    B_b1: jax.Array,
    B_w2: jax.Array,
    B_b2: jax.Array,
):
    del B_x
    bf = jnp.bfloat16
    f32 = jnp.float32
    any_spec = pl.BlockSpec(memory_space=pl.ANY)
    out = pl.pallas_call(
        _kernel,
        out_shape=jax.ShapeDtypeStruct((S, D), bf),
        in_specs=[any_spec] * 7,
        out_specs=any_spec,
        scratch_shapes=[
            pltpu.VMEM((S, D), bf),
            pltpu.VMEM((S, D), bf),
            pltpu.VMEM((SUB, D), bf),
            pltpu.VMEM((D, 3 * D), bf),
            pltpu.VMEM((D, D), bf),
            pltpu.VMEM((D, F), bf),
            pltpu.VMEM((F, D), bf),
            pltpu.VMEM((24, S, 128), bf),
            pltpu.VMEM((D, S), bf),
            pltpu.VMEM((HB * NSUB, 128 + ZP, TQ), bf),
            pltpu.VMEM((D, S), bf),
            pltpu.VMEM((D - HB * DH, S), bf),
            pltpu.VMEM((HB * DH, S), bf),
            pltpu.VMEM((S, KP), bf),
            pltpu.VMEM((HB * NSUB, S, TQ), f32),
            pltpu.VMEM((HB * NSUB, 8, TQ), f32),
            pltpu.VMEM((TM3, D), bf),
            pltpu.VMEM((TM3, D), f32),
            pltpu.VMEM((S, D), f32),
            pltpu.VMEM((2, TM3, D), bf),
            pltpu.VMEM((1, F), f32),
            pltpu.VMEM((1, D), f32),
            pltpu.VMEM((F // 128, 128), bf),
            pltpu.VMEM((D // 128, 128), bf),
            pltpu.SemaphoreType.DMA((NX + 1,)),
            pltpu.SemaphoreType.DMA((NWC + 1,)),
            pltpu.SemaphoreType.DMA((5,)),
            pltpu.SemaphoreType.DMA((2,)),
        ],
        compiler_params=pltpu.CompilerParams(
            vmem_limit_bytes=120 * 1024 * 1024,
            internal_scratch_in_bytes=65536,
        ),
    )(A_x.reshape(S, D), A_wqkv, A_wo, B_w1, B_b1.reshape(F // 128, 128), B_w2,
      B_b2.reshape(D // 128, 128))
    return out.reshape(1, S, D)
```

```python
import math

import jax
import jax.numpy as jnp
from jax import lax
import jax.experimental.pallas as pl
import jax.experimental.pallas.tpu as pltpu

S = 2048
D = 1024
H = 32
DH = 32
F = 3584
EPS = 1e-5
NT = (((1,), (1,)), ((), ()))
QSCALE = (DH ** -0.5) * math.log2(math.e)

TX = 256
NX = S // TX
SUB = 128
WC = 512
NWC = 3 * D // WC
TB = 1024
TQ = 512
NSUB = S // TQ
TK = 128
NC = S // TK
HB = 2
LAG = 2
ZP = 128 - DH
KP = D - 128
TM3 = 128
N3 = S // TM3
TF = 896
A2_SLOT = 6


def _ln(x):
    m = jnp.mean(x, axis=-1, keepdims=True)
    xc = x - m
    v = jnp.mean(xc * xc, axis=-1, keepdims=True)
    return xc * lax.rsqrt(v + EPS)


def _kernel(x_hbm, wqkv_hbm, wo_hbm, w1_hbm, b1_hbm, w2_hbm, b2_hbm, out_hbm,
            x_v, xn_v, xs_v, wqkv_v, wo_v, w1_v, w2_v, qkv_v, qt_v, qz_v, vt_v,
            ot_v, otl_v, og_v, s_v, m_v, y_v, h_v, hp_v, o_v, b1_v, b2_v,
            b1r_v, b2r_v, x_sems, w_sems, in_sems, out_sems):
    f32 = jnp.float32
    bf16 = jnp.bfloat16

    def x_copy(r0, n, k):
        rows = pl.ds(r0, n)
        return pltpu.make_async_copy(x_hbm.at[rows, :], x_v.at[rows, :], x_sems.at[k])

    def x_mid(i):
        return x_copy(pl.multiple_of(SUB + i * TX, SUB), TX, i + 1)

    def w_copy(c0, n, k):
        cols = pl.ds(c0, n)
        return pltpu.make_async_copy(wqkv_hbm.at[:, cols], wqkv_v.at[:, cols], w_sems.at[k])

    def w_chunk(j):
        return w_copy(pl.multiple_of(j * WC, WC), WC, j)

    cp_wo = pltpu.make_async_copy(wo_hbm, wo_v, in_sems.at[0])
    cp_w1 = pltpu.make_async_copy(w1_hbm, w1_v, in_sems.at[1])
    cp_w2 = pltpu.make_async_copy(w2_hbm, w2_v, in_sems.at[2])
    cp_b1 = pltpu.make_async_copy(b1_hbm, b1r_v, in_sems.at[3])
    cp_b2 = pltpu.make_async_copy(b2_hbm, b2r_v, in_sems.at[4])
    HW = WC // 2
    cp_xa = x_copy(0, TX, 0)
    cp_xb = x_copy(TX, SUB, 1)
    cp_xz = x_copy(S - SUB, SUB, NX)
    cp_w0a = w_copy(0, HW, 0)
    cp_w0b = w_copy(HW, HW, NWC)

    cp_xa.start(); cp_w0a.start(); cp_w0b.start(); cp_xb.start()
    x_mid(1).start()

    for b in range(HB * NSUB):
        qz_v[b, 0:ZP, :] = jnp.zeros((ZP, TQ), bf16)
        qz_v[b, 128:128 + ZP, :] = jnp.zeros((ZP, TQ), bf16)

    def ln_rows(r0):
        rows = pl.ds(pl.multiple_of(r0, SUB), SUB)
        xn = _ln(x_v[rows, :].astype(f32)).astype(bf16)
        xn_v[rows, :] = xn
        return xn

    def q_store(rows, g0, r):
        r = (r * QSCALE).astype(bf16)
        for g in range(r.shape[1] // 128):
            qkv_v[g0 + g, rows, :] = r[:, g * 128:(g + 1) * 128]

    cp_xa.wait()
    ln_rows(0)
    ln_rows(SUB)
    cp_w0a.wait()
    q_store(pl.ds(0, TX), 0,
            jnp.dot(xn_v[0:TX, :], wqkv_v[:, 0:HW], preferred_element_type=f32))
    cp_w0b.wait()
    cp_xb.wait()
    for i in range(2, NX - 1):
        x_mid(i).start()
    cp_xz.start()
    q_store(pl.ds(0, TX), HW // 128,
            jnp.dot(xn_v[0:TX, :], wqkv_v[:, HW:WC], preferred_element_type=f32))
    xs_v[...] = ln_rows(TX)

    def p1a(i, c):
        @pl.when(i < NX - 1)
        def _():
            x_mid(i).wait()

        @pl.when(i == NX - 1)
        def _():
            cp_xz.wait()

        @pl.when(i == 3)
        def _():
            for j in range(1, NWC):
                w_chunk(j).start()

        xn = xs_v[...]
        for u in range(TX // SUB):
            r0 = i * TX + u * SUB
            rows = pl.ds(pl.multiple_of(r0, SUB), SUB)
            r = jnp.dot(xn, wqkv_v[:, 0:WC], preferred_element_type=f32)
            nrows = pl.ds(pl.multiple_of(jnp.minimum(r0 + SUB, S - SUB), SUB), SUB)
            xx = x_v[nrows, :].astype(f32)
            xc = xx - jnp.mean(xx, axis=-1, keepdims=True)
            rs = lax.rsqrt(jnp.mean(xc * xc, axis=-1, keepdims=True) + EPS)
            xn = (xc * rs).astype(bf16)
            xn_v[nrows, :] = xn
            if u == TX // SUB - 1:
                hi = r[:, HW:] * (QSCALE + jnp.minimum(rs, 0.0))
                r = jnp.concatenate([(r[:, 0:HW] * QSCALE).astype(bf16), hi.astype(bf16)],
                                    axis=1)
            else:
                r = (r * QSCALE).astype(bf16)
            for g in range(WC // 128):
                qkv_v[g, rows, :] = r[:, g * 128:(g + 1) * 128]
        xs_v[...] = xn
        return c
    lax.fori_loop(1, NX, p1a, 0)

    nb = S // TB

    def p1b(t, c):
        j = t // nb + 1
        i = t % nb

        @pl.when(i == 0)
        def _():
            w_chunk(j).wait()

        @pl.when(t == 1)
        def _():
            cp_b1.start(); cp_b2.start(); cp_wo.start(); cp_w1.start(); cp_w2.start()

        scale = jnp.where(j < D // WC, QSCALE, 1.0).astype(f32)
        rows = pl.ds(pl.multiple_of(i * TB, TB), TB)
        cols = pl.ds(pl.multiple_of(j * WC, WC), WC)
        r = jnp.dot(xn_v[rows, :], wqkv_v[:, cols], preferred_element_type=f32)
        r = (r * scale).astype(bf16)
        for g in range(WC // 128):
            qkv_v[j * (WC // 128) + g, rows, :] = r[:, g * 128:(g + 1) * 128]
        return c
    lax.fori_loop(0, (NWC - 1) * nb, p1b, 0)

    cp_b1.wait(); cp_b2.wait()
    lane = lax.broadcasted_iota(jnp.int32, (TQ, 128), 1) // DH

    def stage_q(h, t, b):
        cols = pl.ds(pl.multiple_of(t * TQ, TQ), TQ)
        qz_v[b, ZP:128, :] = qt_v[pl.ds(pl.multiple_of(h * DH, DH), DH), cols]

    def softmax_pv_chunk(b, c, m, ls, ot, vrows):
        rows = pl.ds(c * TK, TK)
        sc = s_v[b, rows, :]

        def finish():
            mm = m
            if c >= LAG:
                mm = m + jnp.minimum(ls[c - LAG], 0.0)
            p = jnp.exp2(sc.reshape(TK // 8, 8, TQ) - mm[None])
            cl = jnp.sum(p, axis=0)
            ls.append(cl if c == 0 else ls[-1] + cl)
            o = jnp.dot(vt_v[vrows, rows], p.reshape(TK, TQ).astype(bf16),
                        preferred_element_type=f32)
            return o if ot is None else o + ot
        return finish

    def att_sub(h, t, b, do_pv, first=False):
        hn = h + HB
        koff = hn // 4 + 8
        if do_pv:
            hoff = pl.multiple_of(h * DH, DH)
            m = m_v[b]
            wstart = pl.multiple_of(ZP - DH * (hn % 4), DH)
        else:
            qg = qkv_v[hn // 4, pl.ds(pl.multiple_of(t * TQ, TQ), TQ), :]
            qm = jnp.where(lane == (hn % 4), qg, jnp.zeros_like(qg))
        mx = None
        ls = []
        ot = None
        for c in range(NC):
            rows = pl.ds(c * TK, TK)
            if do_pv:
                finish = softmax_pv_chunk(b, c, m, ls, ot, pl.ds(hoff, DH))
                qk_first = first and c == 0
                if qk_first:
                    st = jnp.dot(qkv_v[koff, rows, :], qz_v[b, pl.ds(wstart, 128), :],
                                 preferred_element_type=f32)
                ot = finish()
                if not qk_first:
                    st = jnp.dot(qkv_v[koff, rows, :], qz_v[b, pl.ds(wstart, 128), :],
                                 preferred_element_type=f32)
            else:
                st = lax.dot_general(qkv_v[koff, rows, :], qm, NT,
                                     preferred_element_type=f32)
            cm = jnp.max(st.reshape(TK // 8, 8, TQ), axis=0)
            mx = cm if mx is None else jnp.maximum(mx, cm)
            s_v[b, rows, :] = st
        m_v[b] = jnp.broadcast_to(jnp.max(mx, axis=0, keepdims=True), (8, TQ))
        if do_pv:
            ot_v[pl.ds(hoff, DH), pl.ds(pl.multiple_of(t * TQ, TQ), TQ)] = (
                ot / jnp.sum(ls[-1], axis=0, keepdims=True)).astype(bf16)

    def p2a(t, c):
        rows = pl.ds(pl.multiple_of(t * TQ, TQ), TQ)
        for g in range(8):
            qt_v[g * 128:(g + 1) * 128, rows] = qkv_v[g, rows, :].T
        for g in range(8):
            vt_v[g * 128:(g + 1) * 128, rows] = qkv_v[16 + g, rows, :].T
        for cc in range(F // 128):
            b1_v[:, cc * 128:(cc + 1) * 128] = b1r_v[cc:cc + 1, :].astype(f32)
        for cc in range(D // 128):
            b2_v[:, cc * 128:(cc + 1) * 128] = b2r_v[cc:cc + 1, :].astype(f32)
        for j in range(HB):
            att_sub(j - HB, t, j * NSUB + t, False)
        for j in range(HB):
            stage_q(HB + j, t, j * NSUB + t)
        return c
    lax.fori_loop(0, NSUB, p2a, 0)

    def p2(b, c):
        for j in range(HB):
            for t in range(NSUB):
                att_sub(b * HB + j, t, j * NSUB + t, True, first=(j == 0 and t == 0))
        for j in range(HB):
            for t in range(NSUB):
                stage_q(jnp.minimum(b * HB + j + 2 * HB, H - 1), t, j * NSUB + t)
        return c
    lax.fori_loop(0, H // HB - 1, p2, 0)

    cp_wo.wait(); cp_w1.wait(); cp_w2.wait()

    NPC = HB * NC // (TQ // 128)
    PN = D // NPC

    def pre_t(t):
        cols = pl.ds(pl.multiple_of(t * TQ, TQ), TQ)
        og_v[cols, :] = ot_v[0:KP, cols].T

    def p25(t, c_):
        o_cur = [None]

        def piece(k):
            r, n = k // NPC, k % NPC
            rows = pl.ds(pl.multiple_of(t * TQ + r * 128, 128), 128)
            if n == 0:
                o_cur[0] = og_v[rows, :]
            cols = pl.ds(n * PN, PN)
            hp = jnp.dot(o_cur[0], wo_v[0:KP, cols], preferred_element_type=f32)
            hp_v[rows, cols] = hp + x_v[rows, cols].astype(f32)

        for j in range(HB):
            b = j * NSUB + t
            r0 = D - (HB - j) * DH
            m = m_v[b]
            ls = []
            ot = None
            for c in range(NC):
                ot = softmax_pv_chunk(b, c, m, ls, ot, pl.ds(r0, DH))()
                piece(j * NC + c)
            otl_v[j * DH:(j + 1) * DH, pl.ds(pl.multiple_of(t * TQ, TQ), TQ)] = (
                ot / jnp.sum(ls[-1], axis=0, keepdims=True)).astype(bf16)
        pre_t(jnp.minimum(t + 1, NSUB - 1))
        return c_
    pre_t(0)
    lax.fori_loop(0, NSUB, p25, 0)

    def out_copy(i, slot):
        rows = pl.ds(pl.multiple_of(i * TM3, TM3), TM3)
        return pltpu.make_async_copy(o_v.at[slot], out_hbm.at[rows, :], out_sems.at[slot])

    def stage_a(i):
        rows = pl.ds(pl.multiple_of(i * TM3, TM3), TM3)
        o = jnp.concatenate([ot_v[KP:D - HB * DH, rows], otl_v[:, rows]], axis=0).T
        h = hp_v[rows, :] + jnp.dot(o, wo_v[KP:D, :], preferred_element_type=f32)
        y_v[...] = _ln(_ln(h)).astype(bf16)
        h_v[...] = h + b2_v[...]

    def p3(i, c):
        slot = i % 2

        @pl.when(i >= 2)
        def _():
            out_copy(i - 2, slot).wait()

        y = y_v[...]
        acc = h_v[...]
        nxt = jnp.minimum(i + 1, N3 - 1)
        for j in range(F // TF):
            cols = pl.ds(j * TF, TF)
            a = jnp.dot(y, w1_v[:, cols], preferred_element_type=f32)
            a = jax.nn.gelu(a + b1_v[:, cols], approximate=True).astype(bf16)
            if 2 * j == A2_SLOT:
                stage_a(nxt)
            acc = acc + jnp.dot(a, w2_v[cols, :], preferred_element_type=f32)
            if 2 * j + 1 == A2_SLOT:
                stage_a(nxt)
        o_v[slot] = acc.astype(bf16)
        out_copy(i, slot).start()
        return c
    stage_a(0)
    lax.fori_loop(0, N3, p3, 0)
    out_copy(N3 - 2, (N3 - 2) % 2).wait()
    out_copy(N3 - 1, (N3 - 1) % 2).wait()


@jax.jit
def pallas_sequential_preLN__softmax_full_mha__mixer_channel_mlp__prompt_kernel(
    A_x: jax.Array,
    A_wqkv: jax.Array,
    A_wo: jax.Array,
    B_x: jax.Array,
    B_w1: jax.Array,
    B_b1: jax.Array,
    B_w2: jax.Array,
    B_b2: jax.Array,
):
    del B_x
    bf = jnp.bfloat16
    f32 = jnp.float32
    any_spec = pl.BlockSpec(memory_space=pl.ANY)
    out = pl.pallas_call(
        _kernel,
        out_shape=jax.ShapeDtypeStruct((S, D), bf),
        in_specs=[any_spec] * 7,
        out_specs=any_spec,
        scratch_shapes=[
            pltpu.VMEM((S, D), bf),
            pltpu.VMEM((S, D), bf),
            pltpu.VMEM((SUB, D), bf),
            pltpu.VMEM((D, 3 * D), bf),
            pltpu.VMEM((D, D), bf),
            pltpu.VMEM((D, F), bf),
            pltpu.VMEM((F, D), bf),
            pltpu.VMEM((24, S, 128), bf),
            pltpu.VMEM((D, S), bf),
            pltpu.VMEM((HB * NSUB, 128 + ZP, TQ), bf),
            pltpu.VMEM((D, S), bf),
            pltpu.VMEM((D - HB * DH, S), bf),
            pltpu.VMEM((HB * DH, S), bf),
            pltpu.VMEM((S, KP), bf),
            pltpu.VMEM((HB * NSUB, S, TQ), f32),
            pltpu.VMEM((HB * NSUB, 8, TQ), f32),
            pltpu.VMEM((TM3, D), bf),
            pltpu.VMEM((TM3, D), f32),
            pltpu.VMEM((S, D), f32),
            pltpu.VMEM((2, TM3, D), bf),
            pltpu.VMEM((1, F), f32),
            pltpu.VMEM((1, D), f32),
            pltpu.VMEM((F // 128, 128), bf),
            pltpu.VMEM((D // 128, 128), bf),
            pltpu.SemaphoreType.DMA((NX + 1,)),
            pltpu.SemaphoreType.DMA((NWC + 1,)),
            pltpu.SemaphoreType.DMA((5,)),
            pltpu.SemaphoreType.DMA((2,)),
        ],
        compiler_params=pltpu.CompilerParams(
            vmem_limit_bytes=120 * 1024 * 1024,
            internal_scratch_in_bytes=65536,
        ),
    )(A_x.reshape(S, D), A_wqkv, A_wo, B_w1, B_b1.reshape(F // 128, 128), B_w2,
      B_b2.reshape(D // 128, 128))
    return out.reshape(1, S, D)
```
